```python
import os as _os
_os.environ.setdefault('JAX_PLATFORMS', 'cpu')
import jax
import jax.numpy as jnp

def _softmax(x, axis=-1):
    return jax.nn.softmax(x, axis=axis)

def _gelu(x):
    return jax.nn.gelu(x, approximate=True)

def _silu(x):
    return jax.nn.silu(x)

def _sigmoid(x):
    return jax.nn.sigmoid(x)

def _layernorm(x, axis=-1, eps=1e-05):
    m = jnp.mean(x, axis=axis, keepdims=True)
    v = jnp.var(x, axis=axis, keepdims=True)
    return (x - m) / jnp.sqrt(v + eps)

def _scatter_add(tgt, idx, src, axis=0):
    return tgt.at[idx].add(src)

def _segment_sum(src, seg, n):
    return jax.ops.segment_sum(src, seg, n)

class _Rng:

    def __init__(self, key):
        self._k = key

    def _next(self):
        self._k, sub = jax.random.split(self._k)
        return sub

    def normal(self, shape):
        return jax.random.normal(self._next(), shape, dtype=jnp.bfloat16)

    def randint(self, lo, hi, shape):
        return jax.random.randint(self._next(), shape, lo, hi, dtype=jnp.int32)

    def uniform(self, shape, lo=0.0, hi=1.0):
        return jax.random.uniform(self._next(), shape, jnp.bfloat16, lo, hi)

    def permutation(self, n):
        return jax.random.permutation(self._next(), n)
kernel_name = 'concat_heads__spectral_gfnet__memory_aug_recurrent_mem_tr__prompt'

def setup_inputs():
    _rng = _Rng(jax.random.key(int.from_bytes(__import__("os").urandom(4), "little")))
    _w = lambda a: (lambda t: t.astype(jnp.bfloat16) if jnp.issubdtype(t.dtype, jnp.floating) else t)(jnp.asarray(a))

    def _A_setup():
        B, S, D = (1, 2048, 512)
        Df = D // 2 + 1
        return {'x': _w((lambda *s: _rng.normal(s) * 0.05)(B, S, D)), 'w_r': _w((lambda *s: _rng.normal(s) * 0.05)(S, Df) * 0.02), 'w_i': _w((lambda *s: _rng.normal(s) * 0.05)(S, Df) * 0.02)}
    _A_in = _A_setup()

    def _B_setup():
        B, S, Dm = (1, 2048, 512)
        H, Dh = (32, 128)
        M, seg = (8, 32)
        seg = min(seg, S)
        S = S // seg * seg
        return {'x': _w((lambda *s: _rng.normal(s) * 0.05)(B, S, Dm)), 'mem0': _w((lambda *s: _rng.normal(s) * 0.4)(B, M, Dm)), 'Wq': _w((lambda *s: _rng.normal(s) * 3.2)(Dm, H, Dh) * Dm ** (-0.5)), 'Wk': _w((lambda *s: _rng.normal(s) * 3.2)(Dm, H, Dh) * Dm ** (-0.5)), 'Wv': _w((lambda *s: _rng.normal(s) * 0.4)(Dm, H, Dh) * Dm ** (-0.5)), 'Wo': _w((lambda *s: _rng.normal(s) * 0.4)(H, Dh, Dm) * (H * Dh) ** (-0.5)), 'seg_len': seg}
    _B_in = _B_setup()
    return {'A_x': _A_in['x'], 'A_w_r': _A_in['w_r'], 'A_w_i': _A_in['w_i'], 'B_x': _B_in['x'], 'B_mem0': _B_in['mem0'], 'B_Wq': _B_in['Wq'], 'B_Wk': _B_in['Wk'], 'B_Wv': _B_in['Wv'], 'B_Wo': _B_in['Wo'], 'B_seg_len': _B_in['seg_len']}

def reference(A_x, A_w_r, A_w_i, B_x, B_mem0, B_Wq, B_Wk, B_Wv, B_Wo, B_seg_len):

    def _A_ref(x, w_r, w_i):
        B, S, D = x.shape
        X = (lambda x, axes=(-2, -1): jnp.fft.rfft2(x.astype(jnp.float32), axes=axes))(x, axes=(-2, -1))
        W = w_r + 1j * w_i
        X = X * W
        y = (lambda x, s, axes=(-2, -1): jnp.fft.irfft2(x, s=s, axes=axes).astype(jnp.bfloat16))(X, (S, D), axes=(-2, -1))
        return y

    def _B_ref(x, mem0, Wq, Wk, Wv, Wo, seg_len):
        B, S, Dm = x.shape
        H, Dh = (Wq.shape[1], Wq.shape[2])
        M = mem0.shape[1]
        scale = Dh ** (-0.5)
        n_seg = S // seg_len
        L = M + seg_len
        idx = jnp.arange(L)
        mask = (idx[:, None] < M) | (idx[:, None] >= idx[None, :])
        mem = mem0
        outs = []
        for s in range(n_seg):
            xs = x[:, s * seg_len:(s + 1) * seg_len, :].copy()
            h = jnp.concatenate([mem, xs], axis=1)
            q = jnp.einsum('btd,dhe->bhte', h, Wq)
            k = jnp.einsum('btd,dhe->bhte', h, Wk)
            v = jnp.einsum('btd,dhe->bhte', h, Wv)
            scores = jnp.einsum('bhqe,bhke->bhqk', q, k) * scale
            scores = jnp.where(mask[None, None], scores, -1000000000.0)
            p = _softmax(scores, axis=-1)
            o = jnp.einsum('bhqk,bhke->bhqe', p, v)
            o = jnp.einsum('bhte,hed->btd', o, Wo)
            mem = o[:, :M, :].copy()
            outs.append(o[:, M:, :])
        return jnp.concatenate(outs, axis=1)
    a = _A_ref(A_x, A_w_r, A_w_i)
    b = _B_ref(B_x, B_mem0, B_Wq, B_Wk, B_Wv, B_Wo, B_seg_len)
    return jnp.concatenate([a, b], axis=-1)
```

```python
import math

import jax
import jax.numpy as jnp
import ml_dtypes
import numpy as np
from jax.experimental import pallas as pl
from jax.experimental.pallas import tpu as pltpu

S, D = 2048, 512
H, DH, M, SEG = 32, 128, 8, 32
L = M + SEG
NSEG = S // SEG
R = 24
G = 4
NG = H // G
LOG2E = math.log2(math.e)
N1, N2 = 32, 64
PITCH = 36
F32, BF16, U32 = jnp.float32, jnp.bfloat16, jnp.uint32


def _fft_consts():
    n = np.arange(D // 2, dtype=np.float64)
    r = np.arange(128, dtype=np.float64)
    alt = 1.0 - 2.0 * (n % 2)
    ae = 2 * np.pi * np.outer(n, 2 * r) / D
    ao = 2 * np.pi * np.outer(n, 2 * r + 1) / D
    fd = np.stack([np.cos(ae), np.cos(ao), -np.sin(ae), -np.sin(ao)])
    fd[2, :, 0] = alt
    fe = np.concatenate([2 * np.cos(ae).T, -2 * np.sin(ae).T], axis=0) / D
    fe[0] = 1.0 / D
    fe[128] = alt / D
    fo = np.concatenate([2 * np.cos(ao).T, -2 * np.sin(ao).T], axis=0) / D
    fi = np.stack([fe[:, :128], fe[:, 128:], fo[:, :128], fo[:, 128:]])

    s1 = np.arange(N1, dtype=np.float64)[:, None, None]
    f2 = np.arange(N2, dtype=np.float64)[None, :, None]
    s2 = np.arange(N2, dtype=np.float64)[None, None, :]
    th = 2 * np.pi * (s2 * f2 / N2 + s1 * f2 / S)
    c, s = np.cos(th), np.sin(th)
    mf = np.concatenate([np.concatenate([c, s], 2), np.concatenate([-s, c], 2)], 1)
    mi = mf.transpose(0, 2, 1) / S

    a = np.arange(N1, dtype=np.float64)
    f1 = np.concatenate([a[0::2], a[1::2]])
    th = 2 * np.pi * np.outer(a, f1) / N1
    c, s = np.cos(th), np.sin(th)
    nq_r = np.zeros((256, 128))
    nq_r[:N1] = np.concatenate([c, -s, -s, c], 1)
    nq_r[128:128 + N1] = np.concatenate([s, c, c, s], 1)
    c, s = c.T, s.T
    nq_q = np.zeros((2, 128, 128))
    nq_q[0, :, :N1] = np.concatenate([c, -s, c, -s], 0)
    nq_q[1, :, :N1] = np.concatenate([s, c, s, c], 0)
    nq = np.concatenate([nq_r, nq_q.reshape(256, 128)], 0)
    ph = 2 * np.pi * np.outer(np.arange(N2), np.arange(N1)) / S
    tw = np.zeros((2, N2, 128))
    tw[0, :, :N1] = np.cos(ph)
    tw[1, :, :N1] = np.sin(ph)
    bf = ml_dtypes.bfloat16
    return fd.astype(bf), fi.astype(bf), mf.astype(bf), mi.astype(bf), nq.astype(bf), tw.astype(np.float32)


_FD, _FI, _MF, _MI, _NQ, _TW = _fft_consts()


def _cadd(a, b):
    return a[0] + b[0], a[1] + b[1]


def _csub(a, b):
    return a[0] - b[0], a[1] - b[1]


def _cmul_root(a, num, den, sign):
    num %= den
    re, im = a
    if num == 0:
        return a
    if 4 * num == den:
        return (-im, re) if sign > 0 else (im, -re)
    if 2 * num == den:
        return -re, -im
    if 4 * num == 3 * den:
        return (im, -re) if sign > 0 else (-im, re)
    c = math.cos(2 * math.pi * num / den)
    s = sign * math.sin(2 * math.pi * num / den)
    if (8 * num) % den == 0:
        if c * s > 0:
            return (re - im) * c, (re + im) * c
        return (re + im) * c, (im - re) * c
    return re * c - im * s, re * s + im * c


def _dft4(x, sign):
    a, b = _cadd(x[0], x[2]), _csub(x[0], x[2])
    c, d = _cadd(x[1], x[3]), _csub(x[1], x[3])
    if sign < 0:
        y1 = (b[0] + d[1], b[1] - d[0])
        y3 = (b[0] - d[1], b[1] + d[0])
    else:
        y1 = (b[0] - d[1], b[1] + d[0])
        y3 = (b[0] + d[1], b[1] - d[0])
    return [_cadd(a, c), y1, _csub(a, c), y3]


def _dft8(x, sign):
    e = _dft4(x[0::2], sign)
    o = _dft4(x[1::2], sign)
    out = [None] * 8
    for j in range(4):
        if j == 2:
            if sign < 0:
                out[2] = (e[2][0] + o[2][1], e[2][1] - o[2][0])
                out[6] = (e[2][0] - o[2][1], e[2][1] + o[2][0])
            else:
                out[2] = (e[2][0] - o[2][1], e[2][1] + o[2][0])
                out[6] = (e[2][0] + o[2][1], e[2][1] - o[2][0])
        else:
            t = _cmul_root(o[j], j, 8, sign)
            out[j] = _cadd(e[j], t)
            out[j + 4] = _csub(e[j], t)
    return out


def _dot(a, b):
    return jnp.dot(a, b, preferred_element_type=F32)


def _ds(start, size):
    return pl.ds(pl.multiple_of(start, size), size)


def _step_order():
    order = []
    for t in range(NG):
        for name, lag in (("Q", 0), ("D", 1), ("V", 0), ("B", 0), ("C", 0), ("E", 3)):
            if 0 <= t - lag < NG:
                order.append((name, t - lag))
    order += [("E", NG - 3), ("D", NG - 1), ("E", NG - 2), ("E", NG - 1)]
    return order


def _kernel(ax_hbm, wr_hbm, wi_hbm, bx_hbm, mem0_hbm, wq_hbm, wk_hbm, wv_hbm, wo_hbm,
            fd_hbm, fi_hbm, mf_hbm, mi_hbm, nq_hbm, tw_hbm,
            out_hbm,
            mem0_ref, nq_ref, tw_ref, wt_s, ax_s, wr_s, wi_s, bx_s, fd_s, fi_s, mf_s, mi_s, raw_s, wqkv_s, wo_s,
            b1_s, b2_s, bt_s, xg_s, g3_s, og_s, mem_s, ya_s, yb_s, sems, *, unroll, phases):

    copies = {}

    def start(name, src, dst):
        cp = pltpu.make_async_copy(src, dst, sems.at[len(copies)])
        cp.start()
        copies[name] = cp

    def wait(*names):
        for n in names:
            copies[n].wait()

    start("ax", ax_hbm, ax_s)
    start("fd", fd_hbm, fd_s)
    start("mf", mf_hbm, mf_s)
    start("bx", bx_hbm, bx_s)
    start("wq", wq_hbm, raw_s.at[0])
    start("wr", wr_hbm, wr_s)
    start("wi", wi_hbm, wi_s)
    start("wk", wk_hbm, raw_s.at[1])
    start("wv", wv_hbm, raw_s.at[2])
    for n in range(4):
        start(f"wo{n}", wo_hbm.at[:, pl.ds(n * 128, 128)], wo_s.at[n])
    start("mi", mi_hbm, mi_s)
    start("fi", fi_hbm, fi_s)
    start("nq", nq_hbm, nq_ref)
    start("tw", tw_hbm, tw_ref)
    start("mem0", mem0_hbm, mem0_ref)

    lane = jax.lax.broadcasted_iota(jnp.int32, (N2, 128), 1)

    wait("ax", "fd")
    RB = 256

    def fft_d_fwd(i, c):
        lo = ax_s[_ds(i * RB, RB), 0:D // 2].astype(F32)
        hi = ax_s[_ds(i * RB, RB), D // 2:D].astype(F32)
        uv = (lo + hi, lo - hi)
        for n in range(4):
            y = _dot(uv[n % 2], fd_s[n])
            for j in range(RB // N1):
                b1_s[n, pl.ds((i * (RB // N1) + j) * PITCH, N1), :] = y[j * N1:(j + 1) * N1]
        return c

    if "fft" in phases:
        jax.lax.fori_loop(0, S // RB, fft_d_fwd, 0)

    wait("mf")
    bt_s[...] = jnp.zeros_like(bt_s)

    def fft_s_fwd(i, c):
        bt = bt_s[...]
        for u in range(4):
            s1 = i * 4 + u
            rows = pl.ds(s1, N2, stride=PITCH)
            m = mf_s[s1]
            for t in range(2):
                re = b1_s[t, rows, :]
                im = b1_s[2 + t, rows, :]
                if t == 0:
                    bt = jnp.where(lane == s1, pltpu.roll(im, s1, 1), bt)
                    im = jnp.where(lane == 0, 0.0, im)
                b2_s[t, s1] = _dot(m, jnp.concatenate([re, im], axis=0).astype(BF16))
        bt_s[...] = bt
        return c

    if "fft" in phases:
        jax.lax.fori_loop(0, N1 // 4, fft_s_fwd, 0)

    def fft_mid(t, g):
        re_rows = _ds(g * 8, 8)
        im_rows = _ds(N2 + g * 8, 8)

        def ld(j):
            return b2_s[t, j, re_rows, :], b2_s[t, j, im_rows, :]

        def st(j, v):
            b2_s[t, j, re_rows, :] = v[0]
            b2_s[t, j, im_rows, :] = v[1]

        for c in range(4):
            y = _dft8([ld(c + 4 * j) for j in range(8)], -1)
            for r in range(8):
                st(c + 4 * r, y[r])
        for r in range(8):
            x = _dft4([_cmul_root(ld(c + 4 * r), c * r, N1, -1) for c in range(4)], -1)
            z = []
            for q in range(4):
                rows = _ds((r + 8 * q) * N2 + g * 8, 8)
                wr, wi = wt_s[0, rows, :], wt_s[1, rows, :]
                if t == 0:
                    wr, wi = wr << 16, wi << 16
                else:
                    wr, wi = wr & U32(0xFFFF0000), wi & U32(0xFFFF0000)
                wr, wi = pltpu.bitcast(wr, F32), pltpu.bitcast(wi, F32)
                z.append((x[q][0] * wr - x[q][1] * wi, x[q][0] * wi + x[q][1] * wr))
            z = _dft4(z, 1)
            for c in range(4):
                st(c + 4 * r, _cmul_root(z[c], c * r, N1, 1))
        for c in range(4):
            y = _dft8([ld(c + 4 * r) for r in range(8)], 1)
            for j in range(8):
                st(c + 4 * j, y[j])

    def fft_nyquist():
        def column(w_ref):
            sub = jax.lax.broadcasted_iota(jnp.int32, (16, 128), 0)
            low = jax.lax.broadcasted_iota(jnp.int32, (16, 128), 1) < 64
            nat = jnp.zeros((16, 128), F32)
            for j in range(16):
                piece = w_ref[256:257, j * 128:(j + 1) * 128].astype(F32)
                nat = jnp.where(sub == j, piece, nat)
            rot = pltpu.roll(nat, 64, 1)
            return jnp.concatenate([jnp.where(low, nat, rot), jnp.where(low, rot, nat)], axis=0)

        wr, wi = column(wr_s), column(wi_s)
        wcat = jnp.concatenate([wr, wr, -wi, wi], axis=0).T[:N2]
        tc, ts = tw_ref[0], tw_ref[1]
        t = _dot(mf_s[0][:, :N2], bt_s[...].astype(BF16))
        tr, ti = t[:N2], t[N2:]
        t2 = jnp.concatenate([tr * tc + ti * ts, ti * tc - tr * ts], axis=1)
        p = _dot(t2, nq_ref[0:256, :]) * wcat
        ur = _dot(p, nq_ref[256:384, :])
        ui = _dot(p, nq_ref[384:512, :])
        u2 = jnp.concatenate([ur * tc - ui * ts, ui * tc + ur * ts], axis=0)
        bt_s[...] = _dot(mi_s[0][:N2, :], u2.astype(BF16))

    wait("bx")

    def gather_g3(i, c):
        a = bx_s[_ds(i * 64 + R, 8), :].astype(F32)
        b = bx_s[_ds(i * 64 + SEG + R, 8), :].astype(F32)
        v = pltpu.bitcast(jnp.concatenate([a, b], axis=0).astype(BF16), U32)
        xg_s[_ds(i * 8, 8), :] = v
        return c

    jax.lax.fori_loop(0, NSEG // 2, gather_g3, 0)

    raw_u = raw_s.bitcast(U32)

    def bulk_qkv(t, c):
        sub = raw_u.at[t, pl.ds(pl.multiple_of(c * 4, 4), D * 16 - 12), :]
        xg = pltpu.bitcast(xg_s[...], BF16)
        for j in range(4):
            a = sub[pl.ds(j, D, stride=16), :]
            for half, w in enumerate((a, a >> 16)):
                w = pltpu.bitcast(w.astype(jnp.uint16), U32)
                idx = t * H + c * 8 + 2 * j + half
                wqkv_s[idx] = w
                g3_s[idx] = _dot(xg, pltpu.bitcast(w, BF16))

    wait("wq", "wr", "wi")

    def w_transpose(i, c):
        cols = _ds(i * 128, 128)
        for n, w_ref in enumerate((wr_s, wi_s)):
            wt_s[n, cols, :] = w_ref.at[pl.ds(0, 256), :].bitcast(U32)[:, cols].T
        return c

    jax.lax.fori_loop(0, S // 128, w_transpose, 0)

    def bulk_q(c, carry):
        bulk_qkv(0, c)
        if "fft" in phases:
            for u in range(2):
                for t in range(2):
                    fft_mid(t, c * 2 + u)
        return carry

    jax.lax.fori_loop(0, 4, bulk_q, 0)
    wait("wk")
    jax.lax.fori_loop(0, 4, lambda c, carry: bulk_qkv(1, c), None)
    wait("wv")
    jax.lax.fori_loop(0, 4, lambda c, carry: bulk_qkv(2, c), None)

    wait("mi", "fi", "nq", "tw", "mem0")
    if "fft" in phases:
        fft_nyquist()

    def fft_s_inv(i, c):
        bt = bt_s[...]
        for u in range(4):
            s1 = i * 4 + u
            rows = pl.ds(s1, N2, stride=PITCH)
            m = mi_s[s1]
            for t in range(2):
                y = _dot(m, b2_s[t, s1].astype(BF16))
                im = y[N2:]
                if t == 0:
                    im = jnp.where(lane == 0, pltpu.roll(bt, 128 - s1, 1), im)
                b1_s[t, rows, :] = y[:N2]
                b1_s[2 + t, rows, :] = im
        return c

    def fft_d_inv(i, c):
        def rows(n):
            return jnp.concatenate([b1_s[n, pl.ds((i * (RB // N1) + j) * PITCH, N1), :]
                                    for j in range(RB // N1)], axis=0)
        ye = jnp.concatenate([rows(0), rows(2)], axis=1)
        yo = jnp.concatenate([rows(1), rows(3)], axis=1)
        for n in range(2):
            e, o = _dot(ye, fi_s[n]), _dot(yo, fi_s[2 + n])
            ya_s[_ds(i * RB, RB), n * 128:(n + 1) * 128] = (e + o).astype(BF16)
            ya_s[_ds(i * RB, RB), (n + 2) * 128:(n + 3) * 128] = (e - o).astype(BF16)
        return c

    if "fft" in phases:
        jax.lax.fori_loop(0, N1 // 4, fft_s_inv, 0)
        jax.lax.fori_loop(0, S // RB, fft_d_inv, 0)
    start("ya", ya_s, out_hbm.at[:, pl.ds(0, D)])

    wait("wo0", "wo1", "wo2", "wo3")
    wo_u = wo_s.bitcast(U32)
    mem_s[...] = mem0_ref[...].astype(F32)
    row = jax.lax.broadcasted_iota(jnp.int32, (L, L), 0)
    col = jax.lax.broadcasted_iota(jnp.int32, (L, L), 1)
    mask = (row < M) | (row >= col)
    scale = DH ** -0.5 * LOG2E
    order = _step_order()

    def step(s, mem):
        xs = bx_s[_ds(s * SEG, SEG), :].astype(F32)
        h = jnp.concatenate([xs[:R], mem], axis=0)
        r8 = _ds(s * 8, 8)
        qkv = ({}, {}, {})
        sc, p, rl, o = {}, {}, {}, {}
        acc = [None] * 4

        def proj(t, hh):
            y = _dot(h, pltpu.bitcast(wqkv_s[t * H + hh], BF16))
            qkv[t][hh] = jnp.concatenate([y[R:], y[:R], g3_s[t * H + hh, r8, :]], axis=0)

        def stage(name, g):
            heads = range(g * G, g * G + G)
            if name == "Q":
                for hh in heads:
                    proj(0, hh)
                    proj(1, hh)
            elif name == "V":
                for hh in heads:
                    proj(2, hh)
            elif name == "B":
                for hh in heads:
                    sc[hh] = jax.lax.dot_general(qkv[0][hh] * scale, qkv[1][hh], (((1,), (1,)), ((), ())),
                                                 preferred_element_type=F32)
            elif name == "C":
                for hh in heads:
                    z = jnp.where(mask, sc[hh], -1e9 * LOG2E)
                    e = jnp.exp2(z - jnp.max(z, axis=1, keepdims=True))
                    p[hh] = e
                    rl[hh] = pltpu.reciprocal(jnp.sum(e, axis=1, keepdims=True), approx=True)
            elif name == "D":
                for hh in heads:
                    y = _dot(p[hh], qkv[2][hh]) * rl[hh]
                    o[hh] = y[:M + R]
                    og_s[hh, r8, :] = y[M + R:]
            elif name == "E":
                oc = jnp.concatenate([o[hh] for hh in heads], axis=1)
                for n in range(4):
                    y = _dot(oc, pltpu.bitcast(wo_u[n, pl.ds(g * G * 64, G * 64), :], BF16))
                    acc[n] = y if acc[n] is None else acc[n] + y

        for name, g in order:
            stage(name, g)
        out = jnp.concatenate(acc, axis=1)
        yb_s[pl.ds(pl.multiple_of(s * SEG, SEG), 16), :] = out[M:M + 16].astype(BF16)
        yb_s[_ds(s * SEG + 16, 8), :] = out[M + 16:].astype(BF16)
        return out[:M]

    def body(i, c):
        mem = mem_s[...]
        for u in range(unroll):
            mem = step(i * unroll + u, mem)
        mem_s[...] = mem
        return c

    if "rec" in phases:
        jax.lax.fori_loop(0, NSEG // unroll, body, 0)

    OB = 128
    for c in range(NSEG * 8 // OB):
        def bulk_o(c=c):
            oc = jnp.concatenate([og_s[hh, pl.ds(c * OB, OB), :] for hh in range(H)], axis=1)
            for n in range(4):
                y = _dot(oc, pltpu.bitcast(wo_u[n], BF16))
                for j in range(OB // 8):
                    yb_s[pl.ds((c * (OB // 8) + j) * SEG + R, 8), n * 128:(n + 1) * 128] = (
                        y[j * 8:(j + 1) * 8].astype(BF16))
        if "out" in phases:
            bulk_o()
        rows = pl.ds(c * (OB // 8) * SEG, (OB // 8) * SEG)
        start(f"yb{c}", yb_s.at[rows, :], out_hbm.at[rows, pl.ds(D, D)])
    wait("ya", *[f"yb{c}" for c in range(NSEG * 8 // OB)])


def run(A_x, A_w_r, A_w_i, B_x, B_mem0, B_Wq, B_Wk, B_Wv, B_Wo, unroll=2, phases=("fft", "rec", "out")):
    import functools
    any_spec = pl.BlockSpec(memory_space=pltpu.HBM)
    vmem_spec = pl.BlockSpec(memory_space=pltpu.VMEM)
    out = pl.pallas_call(
        functools.partial(_kernel, unroll=unroll, phases=phases),
        out_shape=jax.ShapeDtypeStruct((S, 2 * D), BF16),
        in_specs=[any_spec] * 15,
        out_specs=any_spec,
        scratch_shapes=[
            pltpu.VMEM((M, D), BF16),
            pltpu.VMEM((512, 128), BF16),
            pltpu.VMEM((2, N2, 128), F32),
            pltpu.VMEM((2, S, 128), U32),
            pltpu.VMEM((S, D), BF16),
            pltpu.VMEM((D // 2 + 1, S), BF16),
            pltpu.VMEM((D // 2 + 1, S), BF16),
            pltpu.VMEM((S, D), BF16),
            pltpu.VMEM((4, D // 2, 128), BF16),
            pltpu.VMEM((4, D // 2, 128), BF16),
            pltpu.VMEM((N1, 128, 128), BF16),
            pltpu.VMEM((N1, 128, 128), BF16),
            pltpu.VMEM((3, D * H, DH), BF16),
            pltpu.VMEM((3 * H, D // 2, DH), U32),
            pltpu.VMEM((4, H * DH, 128), BF16),
            pltpu.VMEM((4, N2 * PITCH, 128), F32),
            pltpu.VMEM((2, N1, 128, 128), F32),
            pltpu.VMEM((N2, 128), F32),
            pltpu.VMEM((NSEG * 4, D), U32),
            pltpu.VMEM((3 * H, NSEG * 8, DH), F32),
            pltpu.VMEM((H, NSEG * 8, DH), F32),
            pltpu.VMEM((M, D), F32),
            pltpu.VMEM((S, D), BF16),
            pltpu.VMEM((S, D), BF16),
            pltpu.SemaphoreType.DMA((32,)),
        ],
        compiler_params=pltpu.CompilerParams(vmem_limit_bytes=128 * 1024 * 1024),
    )(A_x.reshape(S, D), A_w_r.T, A_w_i.T, B_x.reshape(S, D), B_mem0.reshape(M, D),
      B_Wq.reshape(D * H, DH), B_Wk.reshape(D * H, DH), B_Wv.reshape(D * H, DH), B_Wo.reshape(H * DH, D),
      _FD, _FI, _MF, _MI, _NQ, _TW)
    return out.reshape(1, S, 2 * D)


@jax.jit
def pallas_concat_heads__spectral_gfnet__memory_aug_recurrent_mem_tr__prompt_kernel(
    A_x, A_w_r, A_w_i, B_x, B_mem0, B_Wq, B_Wk, B_Wv, B_Wo, B_seg_len,
):
    del B_seg_len
    return run(A_x, A_w_r, A_w_i, B_x, B_mem0, B_Wq, B_Wk, B_Wv, B_Wo)
```

```python
import itertools
import math

import jax
import jax.numpy as jnp
import numpy as np
from jax.experimental import pallas as pl
from jax.experimental.pallas import tpu as pltpu

S, D = 2048, 512
H, DH, M, SEG = 32, 128, 8, 32
L = M + SEG
NSEG = S // SEG
R = 24
NB = NSEG * (SEG - R)
G = 4
NG = H // G
U = 4
PHASE = NSEG // 4
LOG2E = math.log2(math.e)
N1, N2 = 32, 64
PITCH = 12
SLAB = N2 * PITCH
PLANE = 4 * SLAB
RB = 256
KW = 128 * H // 2
F32, BF16, U32 = jnp.float32, jnp.bfloat16, jnp.uint32

SUMS = 4 * 2 * 128
XA0 = (3 * H + 4) * 256
KS0 = XA0 + 14 * 128
WT0 = KS0 + 2 * SUMS
XP0 = WT0 + 2 * S
WORDS = XP0 + 4 * NB // 2
FD0 = NG * SUMS
SP0 = 3 * H * NB
TMP0 = SP0 + 4 * PLANE
WORK = TMP0 + 16 * N2


def _dft_tables():
    bf16 = np.dtype(BF16)
    word = np.concatenate([np.arange(0, 128, 2), np.arange(1, 128, 2)])
    n = np.arange(D // 2)
    even = 2 * np.pi * np.outer(n[:128], 2 * word) / D
    odd = 2 * np.pi * np.outer(n, 2 * word + 1) / D
    c, s = np.cos(even), -np.sin(even)
    f0 = np.concatenate([c[:, :64], s[:, :64]], axis=1)
    f2 = np.concatenate([s[:, 64:], c[:, 64:]], axis=1)
    f0[:, 64] = 1.0 - 2.0 * (n[:128] % 2)
    fwd = np.concatenate([f0, f2, np.cos(odd), -np.sin(odd)], axis=0)
    i0 = 2 * f0.T
    i0[[0, 64]] /= 2
    io = np.concatenate([2 * np.cos(odd).T, -2 * np.sin(odd).T], axis=0)
    inv = np.concatenate([i0, 2 * f2.T, io[:, :128], io[:, 128:]], axis=0) / (D * S)

    ph = 2 * np.pi * np.outer(np.arange(N2), np.arange(N1)) / S
    grouped = ph.reshape(N2 // 8, 8, N1).transpose(0, 2, 1)
    tab = np.broadcast_to(np.stack([np.cos(grouped), np.sin(grouped)]).reshape(2, S, 1), (2, S, 128))

    a = np.arange(N1)
    th = 2 * np.pi * np.outer(a, np.concatenate([a[0::2], a[1::2]])) / N1
    c, s = np.cos(th), np.sin(th)
    nq = np.zeros((704, 128))
    nq[0:N1] = np.concatenate([c, -s, -s, c], axis=1)
    nq[128:128 + N1] = np.concatenate([s, c, c, s], axis=1)
    nq[256:384, :N1] = np.concatenate([c.T, -s.T, c.T, -s.T], axis=0)
    nq[384:512, :N1] = np.concatenate([s.T, c.T, s.T, c.T], axis=0)
    th = 2 * np.pi * np.outer(np.arange(N2), np.arange(N2)) / N2
    nq[512:640, :N2] = np.concatenate([np.cos(th), -np.sin(th)], axis=0)
    nq[640:704] = np.concatenate([np.cos(th), -np.sin(th)], axis=1)
    tw = np.zeros((2, N2, 128))
    tw[0, :, :N1] = np.cos(ph)
    tw[1, :, :N1] = np.sin(ph)
    return fwd.astype(bf16), inv.astype(bf16), tab.astype(np.float32), nq.astype(bf16), tw.astype(np.float32)


_TABLES = _dft_tables()


def _cadd(a, b):
    return a[0] + b[0], a[1] + b[1]


def _csub(a, b):
    return a[0] - b[0], a[1] - b[1]


def _cmul_root(a, num, den, sign):
    num %= den
    re, im = a
    if num == 0:
        return a
    if 4 * num == den:
        return (-im, re) if sign > 0 else (im, -re)
    if 2 * num == den:
        return -re, -im
    if 4 * num == 3 * den:
        return (im, -re) if sign > 0 else (-im, re)
    c = math.cos(2 * math.pi * num / den)
    s = sign * math.sin(2 * math.pi * num / den)
    if (8 * num) % den == 0:
        if c * s > 0:
            return (re - im) * c, (re + im) * c
        return (re + im) * c, (im - re) * c
    return re * c - im * s, re * s + im * c


def _dft4(x, sign):
    a, b = _cadd(x[0], x[2]), _csub(x[0], x[2])
    c, d = _cadd(x[1], x[3]), _csub(x[1], x[3])
    y1 = (b[0] + d[1], b[1] - d[0])
    y3 = (b[0] - d[1], b[1] + d[0])
    if sign > 0:
        y1, y3 = y3, y1
    return [_cadd(a, c), y1, _csub(a, c), y3]


def _dft8(load, store, sign):
    e = _dft4([load(j) for j in range(0, 8, 2)], sign)
    yield
    o = _dft4([load(j) for j in range(1, 8, 2)], sign)
    for j in range(4):
        if j == 2:
            lo = (e[2][0] + o[2][1], e[2][1] - o[2][0])
            hi = (e[2][0] - o[2][1], e[2][1] + o[2][0])
            if sign > 0:
                lo, hi = hi, lo
        else:
            t = _cmul_root(o[j], j, 8, sign)
            lo, hi = _cadd(e[j], t), _csub(e[j], t)
        store(j, lo)
        store(j + 4, hi)
    yield


def _dot(a, b):
    return jnp.dot(a, b, preferred_element_type=F32)


def _dot_nt(a, b):
    return jax.lax.dot_general(a, b, (((1,), (1,)), ((), ())), preferred_element_type=F32)


def _ds(start, size, align=None):
    if isinstance(start, int):
        return pl.ds(start, size)
    return pl.ds(pl.multiple_of(start, align or size), size)


def _packed(words):
    return pltpu.bitcast(words, BF16)


def _split_heads(words):
    return [pltpu.bitcast(w.astype(jnp.uint16), U32) for w in (words, words >> 16)]


def _spread(side, pieces, calls):
    count = itertools.count(1)

    def advance():
        n = next(count)
        for _ in range(n * pieces // calls - (n - 1) * pieces // calls):
            next(side)

    return advance


_PLAIN = {1: (0, 0), 2: (1, 0), 3: (1, 1)}
_SUMMED = (5, 6, 7, 4)


def _row_operands(a11, a12, a21, a22):
    s1 = a21 + a22
    s2 = s1 - a11
    return {1: a11, 2: a12, 3: a12 - s2, 4: a22, 5: s1, 6: s2, 7: a11 - a21}


def _weight_sums(b11, b12, b21, b22):
    t1 = b12 - b11
    t2 = b22 - t1
    return t1, t2, b22 - b12, t2 - b21


def _strassen(product, emit):
    m1 = product(1)
    emit(11, m1 + product(2))
    u2 = m1 + product(6)
    m5 = product(5)
    emit(12, u2 + m5 + product(3))
    u3 = u2 + product(7)
    emit(22, u3 + m5)
    emit(21, u3 - product(4))


_ORDERS = (
    "Q0.v0.B0.C0.Q1.v1.B1.C1.k3.D0.Q2.D1.v2.B2.C2.q3.v3.B3.C3.D2.Q4.D3.v4.B4."
    "C4.Q5.D4.E0.E1.B5.C5.v5.Q6.E2.D5.v6.B6.C6.E3.Q7.D6.v7.B7.C7.E4.E5.D7.E6.E7",
    "y0.q0.v0.B0.C0.Q1.v1.B1.C1.Q2.D1.v2.B2.C2.D0.Q3.v3.B3.C3.D2.Q4.E0.D3.v4."
    "B4.C4.Q5.D4.v5.B5.C5.E1.E2.Q6.D5.v6.B6.C6.E3.Q7.D6.v7.B7.C7.E5.E4.D7.E6.E7",
    "y0.q0.v0.B0.C0.Q1.v1.B1.C1.D0.Q2.D1.v2.B2.C2.Q3.D2.v3.B3.C3.Q4.D3.E0.v4.B4.C4."
    "Q5.D4.v5.B5.C5.b2.a2.Q6.c2.d2.v6.D5.E1.B6.C6.E3.Q7.D6.v7.B7.C7.E4.E5.D7.E6.E7",
    "y0.q0.v0.B0.C0.Q1.v1.B1.C1.D0.Q2.D1.v2.B2.C2.Q3.D2.v3.B3.C3.Q4.D3.v4.E0."
    "B4.C4.Q5.D4.v5.E1.v6.B5.C5.Q6.D5.E2.E3.B6.C6.Q7.D6.v7.B7.C7.E5.D7.E6.E7.E4",
)
_FILTER_ORDERS = (
    "Q0.v0.Q1.B0.C0.v1.B1.C1.k3.D0.Q2.D1.v2.q3.B2.C2.v3.B3.C3.D2.Q4.D3.v4.E0."
    "B4.C4.Q5.D4.E1.B5.C5.E2.v5.Q6.D5.v6.B6.C6.E3.Q7.D6.v7.B7.C7.E5.E4.D7.E6.E7",
    "y0.k1.q1.q0.v0.v1.B0.C0.B1.C1.Q2.D1.v2.B2.C2.D0.Q3.v3.D2.B3.C3.Q4.E0.D3.v4."
    "B4.C4.Q5.D4.v5.Q6.B5.C5.E2.D5.E1.v6.B6.C6.E3.Q7.D6.v7.B7.C7.E5.E4.D7.E6.E7",
    "y0.q0.v0.B0.C0.Q1.v1.B1.C1.D0.Q2.v2.D1.B2.C2.Q3.D2.v3.B3.C3.k4.q4.D3.E0.v4.B4."
    "C4.Q5.D4.v5.B5.C5.b2.d2.c2.a2.Q6.v6.D5.E1.B6.C6.E3.Q7.D6.v7.B7.C7.E4.E5.D7.E6.E7",
    "y0.q0.v0.B0.C0.Q1.v1.B1.C1.D0.Q2.D1.v2.B2.C2.Q3.D2.v3.B3.C3.Q4.D3.v4.B4."
    "C4.Q5.D4.v5.E0.v6.E2.B5.C5.E1.Q6.D5.E3.B6.C6.Q7.D6.v7.B7.C7.E5.D7.E6.E7.E4",
)


def _kernel(ax_hbm, wr_hbm, wi_hbm, bx_hbm, mem0_hbm, wq_hbm, wk_hbm, wv_hbm, wo_hbm,
            fwd_hbm, inv_hbm, tab_hbm, nq_hbm, tw_hbm, zero_ref,
            out_hbm,
            nq_s, tw_s, ax_s, w_s, bx_s, inv_s, tab_s, raw_s, words_s, wo_s, ws_s,
            nyq_s, xg_s, work_s, mem_s, ya_s, yb_s, mem0_s, wn_s, sems):
    copies = {}

    def start(name, src, dst):
        copies[name] = pltpu.make_async_copy(src, dst, sems.at[11 + len(copies)])
        copies[name].start()

    def wait(*names):
        for name in names:
            copies[name].wait()

    def xg_copy(kt):
        return pltpu.make_async_copy(
            bx_hbm.at[:, pl.ds(R, SEG - R), _ds(kt * 128, 128)], xg_s.at[kt], sems.at[kt])

    def wq_copy(kt):
        return pltpu.make_async_copy(
            wq_hbm.at[_ds(kt * 2 * KW, 2 * KW), :], raw_s.at[0, _ds(kt * 2 * (KW + 32), 2 * KW, 64), :],
            sems.at[4 + kt])

    def yb_copy(first, count):
        segs = _ds(first, count)
        return pltpu.make_async_copy(yb_s.at[segs], out_hbm.at[segs, :, pl.ds(D, D)], sems.at[8])

    ya_copy = pltpu.make_async_copy(ya_s, out_hbm.at[:, :, pl.ds(0, D)], sems.at[9])

    for kt in range(4):
        xg_copy(kt).start()
        wq_copy(kt).start()
    start("wk", wk_hbm, raw_s.at[1, pl.ds(0, D * H), :])
    start("wv", wv_hbm, raw_s.at[2, pl.ds(0, D * H), :])
    for n in range(4):
        start(f"wo{n}", wo_hbm.at[:, pl.ds(n * 128, 128)], wo_s.at[n])
    for n, w_hbm in enumerate((wr_hbm, wi_hbm)):
        for blk in range(S // 128):
            pltpu.make_async_copy(w_hbm.at[pl.ds(0, 256), pl.ds(blk * 128, 128)],
                                  w_s.at[pl.ds(2 * (n * S + blk * 128), 256), :], sems.at[10]).start()
        start(f"wn{n}", w_hbm.at[pl.ds(256, 1), :], wn_s.at[n])
    start("fwd", fwd_hbm, ws_s.at[pl.ds(2 * FD0, 768), :])
    start("ax", ax_hbm, ax_s)
    start("mem0", mem0_hbm, mem0_s)
    start("bx0", bx_hbm.at[pl.ds(0, PHASE)], bx_s.at[pl.ds(0, PHASE)])
    start("bx1", bx_hbm.at[pl.ds(PHASE, NSEG - PHASE)], bx_s.at[pl.ds(PHASE, NSEG - PHASE)])
    start("tab", tab_hbm, tab_s)
    start("nq", nq_hbm, nq_s)
    start("tw", tw_hbm, tw_s)
    start("inv", inv_hbm, inv_s)

    zero = zero_ref[0]
    raw_u = raw_s.bitcast(U32)
    wo_u = wo_s.bitcast(U32)
    ws_u = ws_s.bitcast(U32)

    def tail_q(kt, pairs, sides=(), x=None):
        raw = raw_u.at[0, _ds(kt * (KW + 32), KW + 32, 32), :]
        held = words_s.at[_ds(zero + XP0 + kt * 256, 256, 128), :]
        sides = [_spread(side, pieces, len(pairs) * 8) for side, pieces in sides]
        if x is None and not sides:
            x = _packed(held[...])
        for j in pairs:
            for half, w in enumerate(_split_heads(raw[pl.ds(j, 128, stride=16), :])):
                head = 2 * j + half
                words_s[_ds(head * 256 + kt * 64, 64), :] = w
                if sides:
                    parts = []
                    for r in range(0, 256, 64):
                        for side in sides:
                            side()
                        parts.append(held[pl.ds(r, 64), :])
                    x = _packed(jnp.concatenate(parts, axis=0))
                rows = pl.ds(head * NB, NB)
                before = work_s[rows, :]
                if not isinstance(kt, int):
                    before = jnp.where(kt > 0, before, 0.0)
                work_s[rows, :] = before + _dot(x, _packed(w))

    def tail_q_trip(kt, pairs):
        xg_copy(kt).wait()
        wq_copy(kt).wait()
        x = xg_s[kt].reshape(NB, 128)
        words_s[_ds(XP0 + kt * 256, 256, 128), :] = pltpu.bitcast(x, U32)
        tail_q(kt, pairs, x=x)

    jax.lax.fori_loop(0, 3, lambda kt, _: tail_q_trip(kt, range(H // 2)), None)
    tail_q_trip(3, range(8))

    def prepare_rows():
        for r in range(0, 128, 8):
            for n in range(2):
                blocks = [_packed(words_s[pl.ds(XP0 + (2 * k + n) * 256 + half * 128 + r, 8), :]).astype(F32)
                          for half in range(2) for k in range(2)]
                for i, a in _row_operands(*blocks).items():
                    words_s[pl.ds(XA0 + (2 * (i - 1) + n) * 128 + r, 8), :] = pltpu.bitcast(a.astype(BF16), U32)
                yield

    def prepare_kv(i, p):
        src = jnp.minimum(i, 7)
        tiles = words_s.at[_ds((H + i * 8 + 4 * p) * 256, 4 * 256), :]
        for r in range(0, 256, 16):
            for j in range(2):
                blocks = []
                for k in range(2):
                    raw = raw_u.at[1 + src // 4, _ds(src % 4 * 4 + (k * 256 + r) * 16, 260, 4), :]
                    words = raw[pl.ds(2 * p + j, 16, stride=16), :]
                    for half, w in enumerate(_split_heads(words)):
                        tiles[pl.ds((2 * j + half) * 256 + k * 128 + r // 2, 8), :] = w
                    blocks += [pltpu.bitcast(w, F32) for w in (words << 16, words & U32(0xFFFF0000))]
                for slot, w in enumerate(_weight_sums(*blocks)):
                    at = KS0 + p * SUMS + slot * 256 + j * 128 + r // 2
                    words_s[pl.ds(at, 8), :] = pltpu.bitcast(w.astype(BF16), U32)
                yield

    def prepare_wo():
        for g in range(NG):
            for r in range(0, 128, 8):
                for j in range(2):
                    blocks = [_packed(wo_u[2 * half + j, pl.ds(g * 256 + k * 128 + r, 8), :]).astype(F32)
                              for k in range(2) for half in range(2)]
                    for slot, w in enumerate(_weight_sums(*blocks)):
                        ws_s[pl.ds(2 * (g * SUMS + slot * 256 + j * 128 + r), 16), :] = w.astype(BF16)
                    yield

    lane = jax.lax.broadcasted_iota(jnp.int32, (N1, 128), 1)

    def feature_dft(side):
        nyq = jnp.zeros((N1, 128), F32)
        for s2 in range(N2):
            x = [ax_s[pl.ds(s2 * N1, N1), pl.ds(n * 128, 128)].astype(F32) for n in range(4)]
            u, w = x[0] + x[2], x[1] + x[3]
            v = jnp.concatenate([x[0] - x[2], x[1] - x[3]], axis=1)
            y = []
            for rows, at, size in ((u + w, 0, 64), (u - w, 64, 64), (v, 128, 128), (v, 256, 128)):
                side()
                f = jnp.concatenate([ws_u.at[_ds(zero + FD0, 3 * 128, 128), :][pl.ds(at, 8), :],
                                     ws_u[pl.ds(FD0 + at + 8, size - 8), :]], axis=0)
                y.append(_dot(rows, _packed(f)))
            re = jnp.where(lane < 64, y[0], y[1])
            im = pltpu.roll(jnp.where(lane < 64, y[1], y[0]), 64, 1)
            nyq = jnp.where(lane == s2, pltpu.roll(y[0], 64 + s2, 1), nyq)
            im = jnp.where(lane == 0, 0.0, im)
            for n, part in enumerate((re, y[2], im, y[3])):
                for a in range(4):
                    work_s[pl.ds(SP0 + n * PLANE + a * SLAB + s2 * PITCH, 8), :] = part[a * 8:(a + 1) * 8]
        nyq_s[...] = nyq

    wait("wk")
    tail_q(3, range(8, 10), [(prepare_rows(), 32), (prepare_kv(0, 0), 32)])

    def tail_kv(i):
        for p in range(2):
            side = _spread(prepare_kv(i + p, 1 - p), 32, 7 * 16)
            held = words_s.at[_ds(zero + XA0, 14 * 128, 128), :]
            tiles = words_s.at[_ds((H + i * 8 + 4 * p) * 256, 4 * 256), :]
            tails = work_s.at[_ds((H + i * 8 + 4 * p) * NB, 4 * NB), :]
            for r0 in (0, 64):
                def product(n):
                    top = []
                    for r in range(r0, r0 + 64, 8):
                        side()
                        top.append(held[pl.ds(2 * (n - 1) * 128 + r, 8), :])
                    a = jnp.concatenate([_packed(jnp.concatenate(top, axis=0)),
                                         _packed(words_s[pl.ds(XA0 + (2 * n - 1) * 128 + r0, 64), :])], axis=1)
                    if n in _SUMMED:
                        w = [words_s[pl.ds(KS0 + p * SUMS + _SUMMED.index(n) * 256 + j * 128, 128), :]
                             for j in range(2)]
                    else:
                        k, half = _PLAIN[n]
                        w = [tiles[pl.ds((2 * j + half) * 256 + k * 128, 128), :] for j in range(2)]
                    return _dot(a, jnp.concatenate([_packed(x) for x in w], axis=1))

                def emit(ij, v):
                    for j in range(2):
                        at = (2 * j + ij % 10 - 1) * NB + (ij // 10 - 1) * (NB // 2) + 2 * r0
                        tails[pl.ds(at, 128), :] = v[:, j * 128:(j + 1) * 128]

                _strassen(product, emit)

    def tail_kv_trip(i, _):
        tail_kv(2 * i)
        tail_kv(2 * i + 1)

    def tail_kv_part(late, _):
        jax.lax.fori_loop(late, 1 + 3 * late, tail_kv_trip, None)
        pl.when(late == 0)(lambda: wait("wv"))

    jax.lax.fori_loop(0, 2, tail_kv_part, None)

    def transpose_filter():
        words = w_s.bitcast(U32)
        for n in range(2):
            for blk in range(S // 128):
                tile = words.at[pl.ds(n * S + blk * 128, 136), :]
                rows = jnp.concatenate([tile[pl.ds(k, 64, stride=2), :] for k in range(2)], axis=0).T
                for j in range(16):
                    at = WT0 + n * S + j % 8 * 256 + (2 * blk + j // 8) * 8
                    words_s[pl.ds(at, 8), :] = rows[j * 8:(j + 1) * 8]

    filter_rows = w_s.at[pl.ds(0, 4 * S), :]
    pltpu.make_async_copy(filter_rows, filter_rows, sems.at[10]).wait()
    tail_q(3, range(10, 16))
    transpose_filter()
    wait("wo0", "wo1", "wo2", "wo3", "fwd", "ax")
    feature_dft(_spread(prepare_wo(), 32 * NG, 4 * N2))

    def fft_outer(pos, inverse):
        t, a = pos // 4, pos % 4
        slabs = [work_s.at[_ds(SP0 + (t + 2 * (part + inverse - 2 * part * inverse)) * PLANE + a * SLAB, SLAB, 32), :]
                 for part in range(2)]

        def st(j, v):
            for slab, x in zip(slabs, v):
                slab[pl.ds(j * PITCH, 8), :] = x

        def st_tmp(j, v):
            for part in range(2):
                work_s[pl.ds(TMP0 + j * 16 + part * 8, 8), :] = v[part]

        for c in range(8):
            yield from _dft8(lambda j: [slab[pl.ds((c + 8 * j) * PITCH, 8), :] for slab in slabs],
                             lambda r, v: st_tmp(c + 8 * r, v), -1)
        for r in range(8):
            yield from _dft8(
                lambda c: _cmul_root([work_s[pl.ds(TMP0 + (c + 8 * r) * 16 + part * 8, 8), :]
                                      for part in range(2)], c * r, N2, -1),
                lambda q, v: st(r + 8 * q, v), -1)

    def fft_filter(pos):
        t, g = pos % 2, pos // 2
        shift = (16 * (1 - t)).astype(U32)
        planes = [work_s.at[_ds(SP0 + (t + 2 * part) * PLANE + g * 8 * PITCH, 3 * SLAB + 9 * PITCH, 32), :]
                  for part in range(2)]
        filt = [words_s.at[_ds(WT0 + n * S + g * 256, 256, 128), :] for n in range(2)]
        table = [tab_s.at[n, _ds(g * 256, 256), :] for n in range(2)]

        def at(j):
            return pl.ds(j // 8 * SLAB + j % 8, 8, stride=PITCH), slice(None)

        def ld(j):
            return [plane[at(j)] for plane in planes]

        def st(j, v):
            for plane, x in zip(planes, v):
                plane[at(j)] = x

        def twiddle(s1, v, sign):
            if s1 == 0:
                return v
            c, s = (x[pl.ds(s1 * 8, 8), :] for x in table)
            if sign < 0:
                return v[0] * c + v[1] * s, v[1] * c - v[0] * s
            return v[0] * c - v[1] * s, v[1] * c + v[0] * s

        for c in range(4):
            yield from _dft8(lambda j: twiddle(c + 4 * j, ld(c + 4 * j), -1), lambda r, v: st(c + 4 * r, v), -1)
        for r in range(8):
            x = _dft4([_cmul_root(ld(c + 4 * r), c * r, N1, -1) for c in range(4)], -1)
            z = []
            for q in range(4):
                wr, wi = (pltpu.bitcast((w[pl.ds((r + 8 * q) * 8, 8), :] << shift) & U32(0xFFFF0000), F32)
                          for w in filt)
                z.append((x[q][0] * wr - x[q][1] * wi, x[q][0] * wi + x[q][1] * wr))
            z = _dft4(z, 1)
            for c in range(4):
                st(c + 4 * r, _cmul_root(z[c], c * r, N1, 1))
            yield
        for c in range(4):
            yield from _dft8(lambda r: ld(c + 4 * r), lambda j, v: st(c + 4 * j, twiddle(c + 4 * j, v, 1)), 1)

    def filter_nyquist():
        def column(n):
            sub = jax.lax.broadcasted_iota(jnp.int32, (16, 128), 0)
            low = jax.lax.broadcasted_iota(jnp.int32, (16, 128), 1) < 64
            nat = jnp.zeros((16, 128), F32)
            for j in range(16):
                nat = jnp.where(sub == j, wn_s[n, :, j * 128:(j + 1) * 128].astype(F32), nat)
            rot = pltpu.roll(nat, 64, 1)
            return jnp.concatenate([jnp.where(low, nat, rot), jnp.where(low, rot, nat)], axis=0)

        wr, wi = column(0), column(1)
        wcat = jnp.concatenate([wr, wr, -wi, wi], axis=0).T[:N2]
        tc, ts = tw_s[0], tw_s[1]
        b = jnp.concatenate([nyq_s[...], jnp.zeros((128 - N1, 128), F32)], axis=0)
        t = _dot_nt(nq_s[512:640, :], b.astype(BF16))
        yield
        tr, ti = t[:N2], t[N2:]
        p = _dot(jnp.concatenate([tr * tc + ti * ts, ti * tc - tr * ts], axis=1), nq_s[0:256, :]) * wcat
        yield
        ur, ui = _dot(p, nq_s[256:384, :]), _dot(p, nq_s[384:512, :])
        yield
        u2 = jnp.concatenate([ur * tc - ui * ts, ui * tc + ur * ts], axis=0)
        y = _dot(nq_s[640:704, :], u2.astype(BF16))
        yield jnp.concatenate([y, jnp.zeros((N2, 128), F32)], axis=0).T[:N1]

    def plane_rows(n, i, nyq=None):
        parts = []
        for s2 in range(i * (RB // N1), (i + 1) * (RB // N1)):
            part = jnp.concatenate(
                [work_s[pl.ds(SP0 + n * PLANE + a * SLAB + s2 * PITCH, 8), :] for a in range(4)], axis=0)
            if nyq is not None:
                part = jnp.where(lane == 0, pltpu.roll(nyq, 128 - s2, 1) if s2 else nyq, part)
            parts.append(part)
        return jnp.concatenate(parts, axis=0)

    def odd_bins(i):
        y = jnp.concatenate([plane_rows(1, i), plane_rows(3, i)], axis=1)
        return [_dot(y, inv_s[pl.ds(256 + n * 256, 256), :]) for n in range(2)]

    def feature_idft():
        odd = []
        for nyq in filter_nyquist():
            odd.append(odd_bins(len(odd)))
        low = jax.lax.broadcasted_iota(jnp.int32, (RB, 128), 1) < 64
        for i in range(S // RB):
            re, im = plane_rows(0, i), pltpu.roll(plane_rows(2, i, nyq), 64, 1)
            for n, part in ((0, jnp.where(low, re, im)), (2, jnp.where(low, im, re))):
                for j in range(RB // 8):
                    at = SP0 + n * PLANE + j % 4 * SLAB + (i * (RB // N1) + j // 4) * PITCH
                    work_s[pl.ds(at, 8), :] = part[j * 8:(j + 1) * 8]
            if len(odd) < 6:
                odd.append(odd_bins(len(odd)))
        for i in range(S // RB):
            if len(odd) < S // RB:
                odd.append(odd_bins(len(odd)))
            e0 = _dot(plane_rows(0, i), inv_s[0:128, :])
            e2 = _dot(plane_rows(2, i), inv_s[128:256, :])
            segs = pl.ds(i * (RB // SEG), RB // SEG)
            for n, e in enumerate((e0 + e2, e0 - e2)):
                for tile, y in ((n, e + odd[i][n]), (n + 2, e - odd[i][n])):
                    ya_s[segs, :, tile * 128:(tile + 1) * 128] = y.astype(BF16).reshape(RB // SEG, SEG, 128)

    row = jax.lax.broadcasted_iota(jnp.int32, (L, L), 0)
    col = jax.lax.broadcasted_iota(jnp.int32, (L, L), 1)
    mask = (row < M) | (row >= col)
    scale = DH ** -0.5 * LOG2E

    def segments(first, side, pieces, orders):
        fill = _spread(side, pieces, 2 * U * NG)
        tails = [work_s.at[_ds(z + first * 8, (3 * H - 1) * NB + U * 8, 32), :] for z in (0, zero)]
        o_tail = {hh: [] for hh in range(H)}
        mem = mem_s[...]
        outs = []
        for u in range(U):
            h = jnp.concatenate([bx_s[first + u].astype(F32)[:R], mem], axis=0)
            qkv = ({}, {}, {})
            sc, p, rl, o, acc = {}, {}, {}, {}, {}

            def add(key, y):
                acc[key] = acc[key] + y if key in acc else y

            def full(t, hh):
                y = qkv[t][hh]
                return jnp.concatenate(
                    [y[R:], y[:R], tails[t != 1][pl.ds((t * H + hh) * NB + u * 8, 8), :]], axis=0)

            for name, g in ((tok[0], int(tok[1:])) for tok in orders[u].split(".")):
                heads = range(g * G, g * G + G)
                if name in "Qqkv":
                    for t in ((0, 1) if name == "Q" else ("qkv".index(name),)):
                        for hh in heads:
                            qkv[t][hh] = _dot(h, _packed(words_s[pl.ds((t * H + hh) * 256, 256), :]))
                elif name == "y":
                    for kt in range(4):
                        w = [_packed(words_s[pl.ds((H + hh) * 256 + kt * 64, 64), :]) for hh in heads]
                        y = _dot(h[:, kt * 128:(kt + 1) * 128], jnp.concatenate(w, axis=1))
                        for i, hh in enumerate(heads):
                            part = y[:, i * 128:(i + 1) * 128]
                            qkv[1][hh] = part if kt == 0 else qkv[1][hh] + part
                elif name == "B":
                    for hh in heads:
                        sc[hh] = _dot_nt(full(0, hh) * scale, full(1, hh))
                    fill()
                elif name == "C":
                    for hh in heads:
                        z = jnp.where(mask, sc[hh], -1e9 * LOG2E)
                        p[hh] = jnp.exp2(z - jnp.max(z, axis=1, keepdims=True))
                        total = jnp.sum(p[hh], axis=1, keepdims=True)
                        r = pltpu.reciprocal(total, approx=True)
                        rl[hh] = r * (2.0 - total * r)
                elif name == "D":
                    for hh in heads:
                        y = _dot(p[hh], full(2, hh).astype(BF16)) * rl[hh]
                        o[hh] = y[:M + R]
                        o_tail[hh].append(y[M + R:])
                    fill()
                elif u < U - 1:
                    oc = jnp.concatenate([o[hh] for hh in heads], axis=1)
                    for n in (range(4) if name == "E" else ("abcd".index(name),)):
                        add(n, _dot(oc, _packed(wo_u[n, pl.ds(g * 256, 256), :])))
                else:
                    ops = _row_operands(*[
                        jnp.concatenate([rows(hh) for hh in heads[2 * k:2 * k + 2]], axis=1)
                        for rows in (o.get, lambda hh: jnp.concatenate(o_tail[hh], axis=0)) for k in range(2)])

                    def product(n):
                        if n in _SUMMED:
                            w = [ws_u[pl.ds(g * SUMS + _SUMMED.index(n) * 256 + j * 128, 128), :]
                                 for j in range(2)]
                        else:
                            k, half = _PLAIN[n]
                            w = [wo_u[2 * half + j, pl.ds(g * 256 + k * 128, 128), :] for j in range(2)]
                        return _dot(ops[n], jnp.concatenate([_packed(x) for x in w], axis=1))

                    _strassen(product, add)
            out = jnp.concatenate([acc[n] for n in ((0, 1, 2, 3) if u < U - 1 else (11, 12))], axis=1)
            mem = out[:M]
            outs.append(out[M:])
        rest = jnp.concatenate([acc[21], acc[22]], axis=1)
        for u in range(U):
            yb_s[first + u] = jnp.concatenate([outs[u], rest[u * 8:(u + 1) * 8]], axis=0).astype(BF16)
        mem_s[...] = mem
        yb_copy(first, U).start()

    def phase(p, _):
        def outer_trip(i, _):
            side = itertools.chain(*[fft_outer(2 * i + n, p % 2) for n in range(2)])
            segments(jnp.where(p > 0, p + 1, 0) * PHASE + i * U, side, 64, _ORDERS)

        def filter_trip(i, _):
            side = itertools.chain(*[fft_filter(4 * i + n) for n in range(4)])
            segments(PHASE + i * U, side, 96, _FILTER_ORDERS)

        jax.lax.fori_loop(0, PHASE // U, outer_trip, None)

        @pl.when(p == 0)
        def _():
            wait("bx1", "tab")
            jax.lax.fori_loop(0, PHASE // U, filter_trip, None)

        @pl.when(p == 1)
        def _():
            wait("wn0", "wn1", "nq", "tw", "inv")
            feature_idft()
            ya_copy.start()

    wait("mem0", "bx0")
    mem_s[...] = mem0_s[...].astype(F32)
    jax.lax.fori_loop(0, 3, phase, None)
    ya_copy.wait()
    yb_copy(0, NSEG).wait()


@jax.jit
def pallas_concat_heads__spectral_gfnet__memory_aug_recurrent_mem_tr__prompt_kernel(
    A_x, A_w_r, A_w_i, B_x, B_mem0, B_Wq, B_Wk, B_Wv, B_Wo, B_seg_len,
):
    del B_seg_len
    hbm_spec = pl.BlockSpec(memory_space=pltpu.HBM)
    out = pl.pallas_call(
        _kernel,
        out_shape=jax.ShapeDtypeStruct((NSEG, SEG, 2 * D), BF16),
        in_specs=[hbm_spec] * 14 + [pl.BlockSpec(memory_space=pltpu.SMEM)],
        out_specs=hbm_spec,
        scratch_shapes=[
            pltpu.VMEM((704, 128), BF16),
            pltpu.VMEM((2, N2, 128), F32),
            pltpu.VMEM((S, D), BF16),
            pltpu.VMEM((4 * S + 64, 128), BF16),
            pltpu.VMEM((NSEG, SEG, D), BF16),
            pltpu.VMEM((768, 128), BF16),
            pltpu.VMEM((2, S, 128), F32),
            pltpu.VMEM((3, 8 * (KW + 32), DH), BF16),
            pltpu.VMEM((WORDS, 128), U32),
            pltpu.VMEM((4, H * DH, 128), BF16),
            pltpu.VMEM((2 * FD0 + 768, 128), BF16),
            pltpu.VMEM((N1, 128), F32),
            pltpu.VMEM((4, NSEG, SEG - R, 128), BF16),
            pltpu.VMEM((WORK, 128), F32),
            pltpu.VMEM((M, D), F32),
            pltpu.VMEM((NSEG, SEG, D), BF16),
            pltpu.VMEM((NSEG, SEG, D), BF16),
            pltpu.VMEM((M, D), BF16),
            pltpu.VMEM((2, 1, S), BF16),
            pltpu.SemaphoreType.DMA((32,)),
        ],
        compiler_params=pltpu.CompilerParams(vmem_limit_bytes=128 * 1024 * 1024),
    )(A_x.reshape(S, D), A_w_r.T, A_w_i.T, B_x.reshape(NSEG, SEG, D), B_mem0.reshape(M, D),
      B_Wq.reshape(D * H, DH), B_Wk.reshape(D * H, DH), B_Wv.reshape(D * H, DH), B_Wo.reshape(H * DH, D),
      *_TABLES, np.zeros((1,), np.int32))
    return out.reshape(1, S, 2 * D)
```
